```python
import os as _os
_os.environ.setdefault("JAX_PLATFORMS", "cpu")
import jax
import jax.numpy as jnp

def _softmax(x, axis=-1):
    return jax.nn.softmax(x, axis=axis)
def _gelu(x):
    return jax.nn.gelu(x, approximate=True)
def _silu(x):
    return jax.nn.silu(x)
def _sigmoid(x):
    return jax.nn.sigmoid(x)
def _layernorm(x, axis=-1, eps=1e-5):
    m = jnp.mean(x, axis=axis, keepdims=True)
    v = jnp.var(x, axis=axis, keepdims=True)
    return (x - m) / jnp.sqrt(v + eps)
def _scatter_add(tgt, idx, src, axis=0):
    return tgt.at[idx].add(src)
def _segment_sum(src, seg, n):
    return jax.ops.segment_sum(src, seg, n)
class _Rng:
    def __init__(self, key):
        self._k = key
    def _next(self):
        self._k, sub = jax.random.split(self._k)
        return sub
    def normal(self, shape):
        return jax.random.normal(self._next(), shape, dtype=jnp.bfloat16)
    def randint(self, lo, hi, shape):
        return jax.random.randint(self._next(), shape, lo, hi, dtype=jnp.int32)
    def uniform(self, shape, lo=0.0, hi=1.0):
        return jax.random.uniform(self._next(), shape, jnp.bfloat16, lo, hi)
    def permutation(self, n):
        return jax.random.permutation(self._next(), n)


kernel_name = 'parallel_sum__sliding_local_dilated__glu_gated_geglu__prompt'

def setup_inputs():
    _rng = _Rng(jax.random.key(int.from_bytes(__import__("os").urandom(4), "little")))
    _w = (lambda a: (lambda t: t.astype(jnp.bfloat16) if jnp.issubdtype(t.dtype, jnp.floating) else t)(jnp.asarray(a)))
    def _A_setup():
        B, S, D = 1, 2048, 512
        return {
            "x": _w((lambda *s: _rng.normal(s) * 0.05)(B, S, D)),
            "wqkv": _w((lambda *s: _rng.normal(s) * 0.05)(D, 3 * D)),
            "wo": _w((lambda *s: _rng.normal(s) * 0.05)(D, D)),
        }
    _A_in = _A_setup()

    def _B_setup():
        B, S, Dm, Df = 1, 2048, 512, 1376
        return {
            "x": _w((lambda *s: _rng.normal(s) * 0.05)(B, S, Dm)),
            "w_gate": _w((lambda *s: _rng.normal(s) * 0.1)(Dm, Df) * (Dm ** -0.5)),
            "w_up": _w((lambda *s: _rng.normal(s) * 0.1)(Dm, Df) * (Dm ** -0.5)),
            "w_down": _w((lambda *s: _rng.normal(s) * 0.1)(Df, Dm) * (Df ** -0.5)),
        }
    _B_in = _B_setup()

    return {
        "A_x": _A_in["x"],
        "A_wqkv": _A_in["wqkv"],
        "A_wo": _A_in["wo"],
        "B_x": _B_in["x"],
        "B_w_gate": _B_in["w_gate"],
        "B_w_up": _B_in["w_up"],
        "B_w_down": _B_in["w_down"],
    }

def reference(A_x, A_wqkv, A_wo, B_x, B_w_gate, B_w_up, B_w_down):
    def _A_ref(x, wqkv, wo):
        B, S, D = x.shape
        H = 32; Dh = D // H
        W, dil = 8, 2
        qkv = (lambda x, *d: x.transpose(*d))((x @ wqkv).reshape(B, S, 3, H, Dh), 2, 0, 3, 1, 4)
        q, k, v = qkv[0], qkv[1], qkv[2]
        scale = Dh ** -0.5
        pos = jnp.arange(S)
        off = jnp.arange(W) * dil
        idx = pos[:, None] - off[None, :]
        mask = idx >= 0
        idx_c = jnp.where(mask, idx, 0).reshape(-1)
        kg = k[:, :, idx_c, :].reshape(B, H, S, W, Dh)
        vg = v[:, :, idx_c, :].reshape(B, H, S, W, Dh)
        logits = jnp.einsum("bhsd,bhswd->bhsw", q, kg) * scale
        logits = jnp.where(mask[None, None, :, :], logits, -1e9)
        attn = _softmax(logits, axis=-1)
        o = jnp.einsum("bhsw,bhswd->bhsd", attn, vg)
        return (lambda x, *d: x.transpose(*d))(o, 0, 2, 1, 3).reshape(B, S, D) @ wo

    def _B_ref(x, w_gate, w_up, w_down):
        g = jnp.einsum("bsd,df->bsf", x, w_gate)
        u = jnp.einsum("bsd,df->bsf", x, w_up)
        h = _gelu(g) * u
        return jnp.einsum("bsf,fd->bsd", h, w_down)

    x = A_x
    xn = _layernorm(x, axis=-1)
    return x + _A_ref(xn, A_wqkv, A_wo) + _B_ref(xn, B_w_gate, B_w_up, B_w_down)
```

```python
import functools

import jax
import jax.numpy as jnp
from jax import lax
import jax.experimental.pallas as pl
import jax.experimental.pallas.tpu as pltpu

S, D, DF = 2048, 512, 1376
H, DH, W, DIL = 32, 16, 8, 2
HALO = 16
TM = 512
EPS = 1e-5


def _kernel(x_ref, wqkv_ref, wo_ref, wg_ref, wu_ref, wd_ref, o_ref,
            wqkv_p, wo_p, kv_buf):
    i = pl.program_id(0)
    f32, bf16 = jnp.float32, jnp.bfloat16

    @pl.when(i == 0)
    def _():
        r = lax.broadcasted_iota(jnp.int32, (D, D), 0)
        c = lax.broadcasted_iota(jnp.int32, (D, D), 1)
        p = (c == (r % DH) * H + r // DH).astype(f32).astype(bf16)
        for s in range(3):
            wqkv_p[:, s * D:(s + 1) * D] = jnp.dot(
                wqkv_ref[:, s * D:(s + 1) * D], p,
                preferred_element_type=f32).astype(bf16)
        pt = (r == (c % DH) * H + c // DH).astype(f32).astype(bf16)
        wo_p[...] = jnp.dot(pt, wo_ref[...],
                            preferred_element_type=f32).astype(bf16)
        kv_buf[0:HALO, :] = jnp.zeros((HALO, 2 * D), f32)

    x = x_ref[...].astype(f32)
    mean = jnp.mean(x, axis=-1, keepdims=True)
    xc = x - mean
    var = jnp.mean(xc * xc, axis=-1, keepdims=True)
    xn = (xc * lax.rsqrt(var + EPS)).astype(bf16)

    qkv = jnp.dot(xn, wqkv_p[...], preferred_element_type=f32)
    q = qkv[:, :D] * (DH ** -0.5)
    kv_buf[HALO:, :] = qkv[:, D:]

    row = lax.broadcasted_iota(jnp.int32, (TM, 128), 0) + i * TM
    logits = []
    for w in range(W):
        kw = kv_buf[pl.ds(HALO - DIL * w, TM), 0:D]
        p = q * kw
        t = (p[:, 0:128] + p[:, 128:256]) + (p[:, 256:384] + p[:, 384:512])
        t = t + pltpu.roll(t, 64, 1)
        t = t + pltpu.roll(t, 32, 1)
        if w > 0:
            t = jnp.where(row >= DIL * w, t, -1e9)
        logits.append(t)
    m = functools.reduce(jnp.maximum, logits)
    es = [jnp.exp(l - m) for l in logits]
    denom = functools.reduce(lambda a, b: a + b, es)
    inv = 1.0 / denom
    acc = None
    for w in range(W):
        vw = kv_buf[pl.ds(HALO - DIL * w, TM), D:2 * D]
        a = es[w] * inv
        a4 = jnp.concatenate([a, a, a, a], axis=1)
        acc = a4 * vw if acc is None else acc + a4 * vw
    kv_buf[0:HALO, :] = kv_buf[TM:TM + HALO, :]

    attn_out = jnp.dot(acc.astype(bf16), wo_p[...], preferred_element_type=f32)

    g = jnp.dot(xn, wg_ref[...], preferred_element_type=f32)
    u = jnp.dot(xn, wu_ref[...], preferred_element_type=f32)
    h = (jax.nn.gelu(g, approximate=True) * u).astype(bf16)
    ffn_out = jnp.dot(h, wd_ref[...], preferred_element_type=f32)

    o_ref[...] = (x + attn_out + ffn_out).astype(o_ref.dtype)


@jax.jit
def pallas_parallel_sum__sliding_local_dilated__glu_gated_geglu__prompt_kernel(
    A_x: jax.Array,
    A_wqkv: jax.Array,
    A_wo: jax.Array,
    B_x: jax.Array,
    B_w_gate: jax.Array,
    B_w_up: jax.Array,
    B_w_down: jax.Array,
):
    x2 = A_x.reshape(S, D)
    full = lambda shape: pl.BlockSpec(shape, lambda i: (0, 0))
    out = pl.pallas_call(
        _kernel,
        grid=(S // TM,),
        in_specs=[
            pl.BlockSpec((TM, D), lambda i: (i, 0)),
            full((D, 3 * D)),
            full((D, D)),
            full((D, DF)),
            full((D, DF)),
            full((DF, D)),
        ],
        out_specs=pl.BlockSpec((TM, D), lambda i: (i, 0)),
        out_shape=jax.ShapeDtypeStruct((S, D), A_x.dtype),
        scratch_shapes=[
            pltpu.VMEM((D, 3 * D), jnp.bfloat16),
            pltpu.VMEM((D, D), jnp.bfloat16),
            pltpu.VMEM((HALO + TM, 2 * D), jnp.float32),
        ],
        compiler_params=pltpu.CompilerParams(
            dimension_semantics=("arbitrary",),
            vmem_limit_bytes=100 * 1024 * 1024,
        ),
    )(x2, A_wqkv, A_wo, B_w_gate, B_w_up, B_w_down)
    return out.reshape(1, S, D)
```

```python
import functools

import jax
import jax.numpy as jnp
from jax import lax
import jax.experimental.pallas as pl
import jax.experimental.pallas.tpu as pltpu

S, D, DF = 2048, 512, 1376
H, DH, W, DIL = 32, 16, 8, 2
HALO = 16
TM = 512
NB = S // TM
EPS = 1e-5
NT = (((1,), (1,)), ((), ()))
GP = [(0, 384), (384, 512), (896, 480)]


def _swap_rows(a):
    return jnp.swapaxes(a.reshape(H, DH, a.shape[-1]), 0, 1).reshape(a.shape)


def _kernel(x_hbm, wqkv_hbm, wo_hbm, wgt_hbm, wut_hbm, wd_hbm, o_ref,
            x_v, wqkv_v, wo_v, wgt_v, wut_v, wd_v, wqkvt_p, wo_p, kv_buf, xn_buf, sems):
    i = pl.program_id(0)
    f32, bf16 = jnp.float32, jnp.bfloat16

    c_wqkv = pltpu.make_async_copy(wqkv_hbm, wqkv_v, sems.at[0])
    c_wo = pltpu.make_async_copy(wo_hbm, wo_v, sems.at[1])
    c_wgs = [pltpu.make_async_copy(wgt_hbm.at[pl.ds(lo, n), :], wgt_v.at[pl.ds(lo, n), :],
                                   sems.at[5 + NB + j]) for j, (lo, n) in enumerate(GP)]
    c_wu = pltpu.make_async_copy(wut_hbm, wut_v, sems.at[3])
    c_wd = pltpu.make_async_copy(wd_hbm, wd_v, sems.at[4])

    def c_x(b):
        return pltpu.make_async_copy(x_hbm.at[pl.ds(b * TM, TM), :],
                                     x_v.at[pl.ds(b * TM, TM), :], sems.at[5 + b])

    def layernorm(x):
        mean = jnp.mean(x, axis=-1, keepdims=True)
        xc = x - mean
        var = jnp.mean(xc * xc, axis=-1, keepdims=True)
        return (xc * lax.rsqrt(var + EPS)).astype(bf16)

    def body(first):
        if first:
            c_x(0).start()
            c_wgs[0].start()
            for cw in c_wgs[1:]:
                cw.start()
            c_wu.start()
            c_wqkv.start()
            c_wo.start()
            c_wd.start()
            for b in range(1, NB):
                c_x(b).start()
            kv_buf[0:HALO, :] = jnp.zeros((HALO, 2 * D), f32)
            c_x(0).wait()
            pass
            x = x_v[0:TM, :].astype(f32)
            xn = layernorm(x)
        else:
            x = x_v[pl.ds(pl.multiple_of(i * TM, TM), TM), :].astype(f32)
            xn = xn_buf[...]

        if first:
            gs = []
            for j, (lo, n) in enumerate(GP):
                c_wgs[j].wait()
                gs.append(lax.dot_general(xn, wgt_v[lo:lo + n, :], NT, preferred_element_type=f32))
            g = jnp.concatenate(gs, axis=1)
            c_wu.wait()
            ua = lax.dot_general(xn, wut_v[0:768, :], NT, preferred_element_type=f32)
            c_wqkv.wait()
            ub = lax.dot_general(xn, wut_v[768:DF, :], NT, preferred_element_type=f32)
            u = jnp.concatenate([ua, ub], axis=1)
            for s in range(3):
                wt = _swap_rows(wqkv_v[:, s * D:(s + 1) * D].astype(f32).T)
                if s == 0:
                    wt = wt * (DH ** -0.5)
                wqkvt_p[s * D:(s + 1) * D, :] = wt.astype(bf16)
            c_wd.wait()
            c_wo.wait()
            c_x(1).wait()
            qkv = lax.dot_general(xn, wqkvt_p[...], NT, preferred_element_type=f32)
            wo_p[...] = _swap_rows(wo_v[...].astype(f32)).astype(bf16)
            h = (jax.nn.gelu(g, approximate=True) * u).astype(bf16)
            ffn_out = jnp.dot(h, wd_v[...], preferred_element_type=f32)
        else:
            qkv = lax.dot_general(xn, wqkvt_p[...], NT, preferred_element_type=f32)
            g = lax.dot_general(xn, wgt_v[...], NT, preferred_element_type=f32)
            u = lax.dot_general(xn, wut_v[...], NT, preferred_element_type=f32)
        q = qkv[:, :D]
        kv_buf[HALO:, :] = qkv[:, D:]

        row = lax.broadcasted_iota(jnp.int32, (TM, 128), 0)
        logits = [None] * W
        for w in (0, 4, 1, 5, 2, 6, 3, 7):
            kw = kv_buf[pl.ds(HALO - DIL * w, TM), 0:D]
            p = q * kw
            t = (p[:, 0:128] + p[:, 128:256]) + (p[:, 256:384] + p[:, 384:512])
            t = t + pltpu.roll(t, 64, 1)
            t = t + pltpu.roll(t, 32, 1)
            if w > 0 and first:
                t = jnp.where(row >= DIL * w, t, -1e9)
            logits[w] = t
        m = functools.reduce(jnp.maximum, logits)
        es = [jnp.exp(l - m) for l in logits]
        denom = functools.reduce(lambda a, b: a + b, es)
        inv = 1.0 / denom
        acc = None
        for w in (0, 4, 1, 5, 2, 6, 3, 7):
            vw = kv_buf[pl.ds(HALO - DIL * w, TM), D:2 * D]
            a = es[w] * inv
            a4 = jnp.concatenate([a, a, a, a], axis=1)
            acc = a4 * vw if acc is None else acc + a4 * vw
        kv_buf[0:HALO, :] = kv_buf[TM:TM + HALO, :]

        attn_out = jnp.dot(acc.astype(bf16), wo_p[...], preferred_element_type=f32)
        if not first:
            h = (jax.nn.gelu(g, approximate=True) * u).astype(bf16)
            ffn_out = jnp.dot(h, wd_v[...], preferred_element_type=f32)
        o_ref[...] = (x + attn_out + ffn_out).astype(o_ref.dtype)
        nb = jnp.minimum(i + 1, NB - 1)
        xn_buf[...] = layernorm(
            x_v[pl.ds(pl.multiple_of(nb * TM, TM), TM), :].astype(f32))

    @pl.when(jnp.logical_and(i > 0, i + 1 < NB))
    def _():
        c_x(i + 1).wait()

    @pl.when(i == 0)
    def _():
        body(True)

    @pl.when(i > 0)
    def _():
        body(False)


@jax.jit
def pallas_parallel_sum__sliding_local_dilated__glu_gated_geglu__prompt_kernel(
    A_x: jax.Array,
    A_wqkv: jax.Array,
    A_wo: jax.Array,
    B_x: jax.Array,
    B_w_gate: jax.Array,
    B_w_up: jax.Array,
    B_w_down: jax.Array,
):
    x2 = A_x.reshape(S, D)
    hbm = pl.BlockSpec(memory_space=pltpu.MemorySpace.HBM)
    bf16 = jnp.bfloat16
    out = pl.pallas_call(
        _kernel,
        grid=(NB,),
        in_specs=[hbm, hbm, hbm, hbm, hbm, hbm],
        out_specs=pl.BlockSpec((TM, D), lambda i: (i, 0)),
        out_shape=jax.ShapeDtypeStruct((S, D), A_x.dtype),
        scratch_shapes=[
            pltpu.VMEM((S, D), bf16),
            pltpu.VMEM((D, 3 * D), bf16),
            pltpu.VMEM((D, D), bf16),
            pltpu.VMEM((DF, D), bf16),
            pltpu.VMEM((DF, D), bf16),
            pltpu.VMEM((DF, D), bf16),
            pltpu.VMEM((3 * D, D), bf16),
            pltpu.VMEM((D, D), bf16),
            pltpu.VMEM((HALO + TM, 2 * D), jnp.float32),
            pltpu.VMEM((TM, D), bf16),
            pltpu.SemaphoreType.DMA((5 + NB + len(GP),)),
        ],
        compiler_params=pltpu.CompilerParams(
            dimension_semantics=("arbitrary",),
            vmem_limit_bytes=100 * 1024 * 1024,
        ),
    )(x2, A_wqkv, A_wo, B_w_gate.T, B_w_up.T, B_w_down)
    return out.reshape(1, S, D)
```

```python
import functools

import jax
import jax.numpy as jnp
from jax import lax
import jax.experimental.pallas as pl
import jax.experimental.pallas.tpu as pltpu

S, D, DF = 2048, 512, 1376
H, DH, W, DIL = 32, 16, 8, 2
HALO = 16
TM = 512
NB = S // TM
EPS = 1e-5
NT = (((1,), (1,)), ((), ()))
GP = [(0, 384), (384, 512), (896, 480)]
USPLIT = 768
QS = 8
W_ORDER = (0, 4, 1, 5, 2, 6, 3, 7)


def _swap_rows(a):
    return jnp.swapaxes(a.reshape(H, DH, a.shape[-1]), 0, 1).reshape(a.shape)


def _geglu(g, u):
    c0 = 0.7978845608028654
    inner = g * (g * g * (c0 * 0.044715) + c0)
    hx = (g * u) * 0.5
    return hx + hx * jnp.tanh(inner)


def _kernel(x_hbm, wqkv_hbm, wo_hbm, wgt_hbm, wut_hbm, wd_hbm, o_ref,
            x_v, wqkv_v, wo_v, wgt_v, wut_v, wd_v, wqkvt_p, wo_p,
            kv_buf, xn_buf, h_buf, sems):
    i = pl.program_id(0)
    f32, bf16 = jnp.float32, jnp.bfloat16

    c_wqkv = pltpu.make_async_copy(wqkv_hbm, wqkv_v, sems.at[0])
    c_wo = pltpu.make_async_copy(wo_hbm, wo_v, sems.at[1])
    c_wu = pltpu.make_async_copy(wut_hbm, wut_v, sems.at[2])
    c_wd = pltpu.make_async_copy(wd_hbm, wd_v, sems.at[3])
    c_wgs = [pltpu.make_async_copy(wgt_hbm.at[pl.ds(lo, n), :], wgt_v.at[pl.ds(lo, n), :],
                                   sems.at[4 + NB + j]) for j, (lo, n) in enumerate(GP)]

    def c_x(b):
        return pltpu.make_async_copy(x_hbm.at[pl.ds(b * TM, TM), :],
                                     x_v.at[pl.ds(b * TM, TM), :], sems.at[4 + b])

    def layernorm(x):
        mean = jnp.mean(x, axis=-1, keepdims=True)
        xc = x - mean
        var = jnp.mean(xc * xc, axis=-1, keepdims=True)
        return (xc * lax.rsqrt(var + EPS)).astype(bf16)

    def mm(a, b_t):
        return lax.dot_general(a, b_t, NT, preferred_element_type=f32)

    def qkv_proj(xn):
        n = TM // QS
        qkv = jnp.concatenate(
            [mm(xn[hh * n:(hh + 1) * n, :], wqkvt_p[...]) for hh in range(QS)], axis=0)
        kv_buf[HALO:, :] = qkv[:, D:]
        return qkv[:, :D]

    def attention(q, r0, r1, first):
        n = r1 - r0
        q = q[r0:r1, :]
        row = lax.broadcasted_iota(jnp.int32, (n, 128), 0) + r0
        logits = [None] * W
        for w in W_ORDER:
            kw = kv_buf[pl.ds(HALO + r0 - DIL * w, n), 0:D]
            p = q * kw
            t = (p[:, 0:128] + p[:, 128:256]) + (p[:, 256:384] + p[:, 384:512])
            t = t + pltpu.roll(t, 64, 1)
            t = t + pltpu.roll(t, 32, 1)
            if w > 0 and first and r0 < DIL * w:
                t = jnp.where(row >= DIL * w, t, -1e9)
            logits[w] = t
        m = functools.reduce(jnp.maximum, logits)
        es = [jnp.exp(l - m) for l in logits]
        denom = functools.reduce(lambda a, b: a + b, es)
        inv = 1.0 / denom
        acc = None
        for w in W_ORDER:
            vw = kv_buf[pl.ds(HALO + r0 - DIL * w, n), D:2 * D]
            a = es[w]
            a4 = jnp.concatenate([a, a, a, a], axis=1)
            acc = a4 * vw if acc is None else acc + a4 * vw
        acc = acc * jnp.concatenate([inv, inv, inv, inv], axis=1)
        return jnp.dot(acc.astype(bf16), wo_p[...], preferred_element_type=f32)

    def body(first):
        if first:
            c_x(0).start()
            for cw in c_wgs:
                cw.start()
            c_wu.start()
            c_wqkv.start()
            c_wo.start()
            c_wd.start()
            for b in range(1, NB):
                c_x(b).start()
            kv_buf[0:HALO, :] = jnp.zeros((HALO, 2 * D), f32)
            c_x(0).wait()
            x = x_v[0:TM, :].astype(f32)
            xn = layernorm(x)
            gs = []
            for j, (lo, n) in enumerate(GP):
                c_wgs[j].wait()
                gs.append(mm(xn, wgt_v[lo:lo + n, :]))
            g = jnp.concatenate(gs, axis=1)
            c_wu.wait()
            ua = mm(xn, wut_v[0:USPLIT, :])
            h_buf[:, 0:USPLIT] = _geglu(g[:, 0:USPLIT], ua).astype(bf16)
            c_wqkv.wait()
            ub = mm(xn, wut_v[USPLIT:DF, :])
            h_buf[:, USPLIT:DF] = _geglu(g[:, USPLIT:DF], ub).astype(bf16)
            for s in range(3):
                wt = _swap_rows(wqkv_v[:, s * D:(s + 1) * D].astype(f32).T)
                if s == 0:
                    wt = wt * (DH ** -0.5)
                wqkvt_p[s * D:(s + 1) * D, :] = wt.astype(bf16)
            q = mm(xn, wqkvt_p[0:D, :])
            kv_buf[HALO:, 0:D] = mm(xn, wqkvt_p[D:2 * D, :])
            c_wd.wait()
            c_wo.wait()
            c_x(1).wait()
            kv_buf[HALO:, D:2 * D] = mm(xn, wqkvt_p[2 * D:3 * D, :])
            wo_p[...] = _swap_rows(wo_v[...].astype(f32)).astype(bf16)
            ffn_out = jnp.dot(h_buf[...], wd_v[...], preferred_element_type=f32)
            attn_out = attention(q, 0, TM, True)
        else:
            x = x_v[pl.ds(pl.multiple_of(i * TM, TM), TM), :].astype(f32)
            xn = xn_buf[...]
            q = qkv_proj(xn)
            gl, al = [], []
            cuts = [0, 384, 768, 1152, DF]
            for j in range(4):
                gl.append(mm(xn, wgt_v[cuts[j]:cuts[j + 1], :]))
                al.append(attention(q, j * (TM // 4), (j + 1) * (TM // 4), False))
            attn_out = jnp.concatenate(al, axis=0)
            g = jnp.concatenate(gl, axis=1)
            u = mm(xn, wut_v[...])
            h = _geglu(g, u).astype(bf16)
            ffn_out = jnp.dot(h, wd_v[...], preferred_element_type=f32)
        kv_buf[0:HALO, :] = kv_buf[TM:TM + HALO, :]
        o_ref[...] = (x + attn_out + ffn_out).astype(o_ref.dtype)
        nb = jnp.minimum(i + 1, NB - 1)
        xn_buf[...] = layernorm(
            x_v[pl.ds(pl.multiple_of(nb * TM, TM), TM), :].astype(f32))

    @pl.when(jnp.logical_and(i > 0, i + 1 < NB))
    def _():
        c_x(i + 1).wait()

    @pl.when(i == 0)
    def _():
        body(True)

    @pl.when(i > 0)
    def _():
        body(False)


@jax.jit
def pallas_parallel_sum__sliding_local_dilated__glu_gated_geglu__prompt_kernel(
    A_x: jax.Array,
    A_wqkv: jax.Array,
    A_wo: jax.Array,
    B_x: jax.Array,
    B_w_gate: jax.Array,
    B_w_up: jax.Array,
    B_w_down: jax.Array,
):
    x2 = A_x.reshape(S, D)
    hbm = pl.BlockSpec(memory_space=pltpu.MemorySpace.HBM)
    bf16 = jnp.bfloat16
    out = pl.pallas_call(
        _kernel,
        grid=(NB,),
        in_specs=[hbm, hbm, hbm, hbm, hbm, hbm],
        out_specs=pl.BlockSpec((TM, D), lambda i: (i, 0)),
        out_shape=jax.ShapeDtypeStruct((S, D), A_x.dtype),
        scratch_shapes=[
            pltpu.VMEM((S, D), bf16),
            pltpu.VMEM((D, 3 * D), bf16),
            pltpu.VMEM((D, D), bf16),
            pltpu.VMEM((DF, D), bf16),
            pltpu.VMEM((DF, D), bf16),
            pltpu.VMEM((DF, D), bf16),
            pltpu.VMEM((3 * D, D), bf16),
            pltpu.VMEM((D, D), bf16),
            pltpu.VMEM((HALO + TM, 2 * D), jnp.float32),
            pltpu.VMEM((TM, D), bf16),
            pltpu.VMEM((TM, DF), bf16),
            pltpu.SemaphoreType.DMA((4 + NB + len(GP),)),
        ],
        compiler_params=pltpu.CompilerParams(
            dimension_semantics=("arbitrary",),
            vmem_limit_bytes=100 * 1024 * 1024,
        ),
    )(x2, A_wqkv, A_wo, B_w_gate.T, B_w_up.T, B_w_down)
    return out.reshape(1, S, D)
```
